```python
import os as _os
_os.environ.setdefault("JAX_PLATFORMS", "cpu")
import jax
import jax.numpy as jnp

def _softmax(x, axis=-1):
    return jax.nn.softmax(x, axis=axis)
def _gelu(x):
    return jax.nn.gelu(x, approximate=True)
def _silu(x):
    return jax.nn.silu(x)
def _sigmoid(x):
    return jax.nn.sigmoid(x)
def _layernorm(x, axis=-1, eps=1e-5):
    m = jnp.mean(x, axis=axis, keepdims=True)
    v = jnp.var(x, axis=axis, keepdims=True)
    return (x - m) / jnp.sqrt(v + eps)
def _scatter_add(tgt, idx, src, axis=0):
    return tgt.at[idx].add(src)
def _segment_sum(src, seg, n):
    return jax.ops.segment_sum(src, seg, n)
class _Rng:
    def __init__(self, key):
        self._k = key
    def _next(self):
        self._k, sub = jax.random.split(self._k)
        return sub
    def normal(self, shape):
        return jax.random.normal(self._next(), shape, dtype=jnp.bfloat16)
    def randint(self, lo, hi, shape):
        return jax.random.randint(self._next(), shape, lo, hi, dtype=jnp.int32)
    def uniform(self, shape, lo=0.0, hi=1.0):
        return jax.random.uniform(self._next(), shape, jnp.bfloat16, lo, hi)
    def permutation(self, n):
        return jax.random.permutation(self._next(), n)


kernel_name = 'sequential_preLN__sliding_local_dilated__dense_activation_mish__prompt'

def setup_inputs():
    _rng = _Rng(jax.random.key(int.from_bytes(__import__("os").urandom(4), "little")))
    _w = (lambda a: (lambda t: t.astype(jnp.bfloat16) if jnp.issubdtype(t.dtype, jnp.floating) else t)(jnp.asarray(a)))
    def _A_setup():
        B, S, D = 1, 2048, 512
        return {
            "x": _w((lambda *s: _rng.normal(s) * 0.05)(B, S, D)),
            "wqkv": _w((lambda *s: _rng.normal(s) * 0.05)(D, 3 * D)),
            "wo": _w((lambda *s: _rng.normal(s) * 0.05)(D, D)),
        }
    _A_in = _A_setup()

    def _B_setup():
        B, S, D, F = 1, 2048, 512, 1376
        return {
            "x": _w((lambda *s: _rng.normal(s) * 0.05)(B, S, D)),
            "w1": _w((lambda *s: _rng.normal(s) * 1.6)(D, F) * (D ** -0.5)),
            "b1": _w((lambda *s: _rng.normal(s) * 0.1)(F)),
            "w2": _w((lambda *s: _rng.normal(s) * 0.1)(F, D) * (F ** -0.5)),
        }
    _B_in = _B_setup()

    return {
        "A_x": _A_in["x"],
        "A_wqkv": _A_in["wqkv"],
        "A_wo": _A_in["wo"],
        "B_x": _B_in["x"],
        "B_w1": _B_in["w1"],
        "B_b1": _B_in["b1"],
        "B_w2": _B_in["w2"],
    }

def reference(A_x, A_wqkv, A_wo, B_x, B_w1, B_b1, B_w2):
    def _A_ref(x, wqkv, wo):
        B, S, D = x.shape
        H = 32; Dh = D // H
        W, dil = 8, 2
        qkv = (lambda x, *d: x.transpose(*d))((x @ wqkv).reshape(B, S, 3, H, Dh), 2, 0, 3, 1, 4)
        q, k, v = qkv[0], qkv[1], qkv[2]
        scale = Dh ** -0.5
        pos = jnp.arange(S)
        off = jnp.arange(W) * dil
        idx = pos[:, None] - off[None, :]
        mask = idx >= 0
        idx_c = jnp.where(mask, idx, 0).reshape(-1)
        kg = k[:, :, idx_c, :].reshape(B, H, S, W, Dh)
        vg = v[:, :, idx_c, :].reshape(B, H, S, W, Dh)
        logits = jnp.einsum("bhsd,bhswd->bhsw", q, kg) * scale
        logits = jnp.where(mask[None, None, :, :], logits, -1e9)
        attn = _softmax(logits, axis=-1)
        o = jnp.einsum("bhsw,bhswd->bhsd", attn, vg)
        return (lambda x, *d: x.transpose(*d))(o, 0, 2, 1, 3).reshape(B, S, D) @ wo

    def _B_ref(x, w1, b1, w2):
        h = jnp.einsum("bsd,df->bsf", x, w1) + b1
        sp = jnp.log1p(jnp.exp(-jnp.abs(h))) + jnp.where(h > 0, h, jnp.zeros_like(h))
        act = h * jnp.tanh(sp)
        return jnp.einsum("bsf,fd->bsd", act, w2)

    x = A_x
    h = x + _A_ref(_layernorm(x, axis=-1), A_wqkv, A_wo)
    h2 = h + _B_ref(_layernorm(h, axis=-1), B_w1, B_b1, B_w2)
    return h2
```

```python
import functools

import jax
import jax.numpy as jnp
import jax.experimental.pallas as pl
import jax.experimental.pallas.tpu as pltpu

_H = 32
_DH = 16
_W = 8
_DIL = 2
_HALO = 16
_EPS = 1e-5


def _layernorm(x):
    m = jnp.mean(x, axis=-1, keepdims=True)
    xc = x - m
    v = jnp.mean(xc * xc, axis=-1, keepdims=True)
    return xc * jax.lax.rsqrt(v + _EPS)


def _kernel(x_ref, wqkv_ref, wo_ref, w1_ref, b1_ref, w2_ref, o_ref, kv_ref, *, ts, d):
    i = pl.program_id(0)
    nchunk = d // 128

    @pl.when(i == 0)
    def _():
        kv_ref[0:_HALO, :] = jnp.zeros((_HALO, 2 * d), jnp.float32)

    @pl.when(i > 0)
    def _():
        kv_ref[0:_HALO, :] = kv_ref[ts:ts + _HALO, :]

    x = x_ref[...].astype(jnp.float32)
    xn = _layernorm(x).astype(jnp.bfloat16)
    qkv = jnp.dot(xn, wqkv_ref[...], preferred_element_type=jnp.float32)
    q = qkv[:, :d] * (_DH ** -0.5)
    kv_ref[_HALO:_HALO + ts, :] = qkv[:, d:]

    row = i * ts + jax.lax.broadcasted_iota(jnp.int32, (ts, 128), 0)
    logits = []
    for w in range(_W):
        off = _HALO - w * _DIL
        acc = None
        for c in range(nchunk):
            kc = kv_ref[off:off + ts, c * 128:(c + 1) * 128]
            t = q[:, c * 128:(c + 1) * 128] * kc
            acc = t if acc is None else acc + t
        acc = acc + pltpu.roll(acc, 64, 1)
        acc = acc + pltpu.roll(acc, 32, 1)
        if w > 0:
            acc = jnp.where(row >= w * _DIL, acc, -1e9)
        logits.append(acc)
    m = functools.reduce(jnp.maximum, logits)
    ps = [jnp.exp(l - m) for l in logits]
    inv = 1.0 / functools.reduce(lambda a, b: a + b, ps)
    o_chunks = []
    for c in range(nchunk):
        acc = None
        for w in range(_W):
            off = _HALO - w * _DIL
            vc = kv_ref[off:off + ts, d + c * 128:d + (c + 1) * 128]
            t = ps[w] * vc
            acc = t if acc is None else acc + t
        o_chunks.append((acc * inv).astype(jnp.bfloat16))
    o = jnp.concatenate(o_chunks, axis=1)

    h = x + jnp.dot(o, wo_ref[...], preferred_element_type=jnp.float32)

    hn = _layernorm(h).astype(jnp.bfloat16)
    h1 = jnp.dot(hn, w1_ref[...], preferred_element_type=jnp.float32)
    h1 = h1 + b1_ref[...].astype(jnp.float32)
    e = jnp.exp(-jnp.abs(h1))
    e2 = e * e
    pos = h1 >= 0
    num = jnp.where(pos, 1.0 + 2.0 * e, e2 + 2.0 * e)
    den = num + jnp.where(pos, 2.0 * e2, 2.0)
    act = (h1 * num / den).astype(jnp.bfloat16)
    out = h + jnp.dot(act, w2_ref[...], preferred_element_type=jnp.float32)
    o_ref[...] = out.astype(o_ref.dtype)


@jax.jit
def pallas_sequential_preLN__sliding_local_dilated__dense_activation_mish__prompt_kernel(
    A_x: jax.Array,
    A_wqkv: jax.Array,
    A_wo: jax.Array,
    B_x: jax.Array,
    B_w1: jax.Array,
    B_b1: jax.Array,
    B_w2: jax.Array,
):
    b, s, d = A_x.shape
    f = B_w1.shape[1]
    ts = 256
    assert b == 1 and s % ts == 0 and d == _H * _DH

    x2 = A_x.reshape(s, d)
    wqkv = A_wqkv.reshape(d, 3, _H, _DH).transpose(0, 1, 3, 2).reshape(d, 3 * d)
    wo = A_wo.reshape(_H, _DH, d).transpose(1, 0, 2).reshape(d, d)
    b1 = B_b1.reshape(1, f)

    const = lambda i: (0, 0)
    out = pl.pallas_call(
        functools.partial(_kernel, ts=ts, d=d),
        grid=(s // ts,),
        in_specs=[
            pl.BlockSpec((ts, d), lambda i: (i, 0)),
            pl.BlockSpec((d, 3 * d), const),
            pl.BlockSpec((d, d), const),
            pl.BlockSpec((d, f), const),
            pl.BlockSpec((1, f), const),
            pl.BlockSpec((f, d), const),
        ],
        out_specs=pl.BlockSpec((ts, d), lambda i: (i, 0)),
        out_shape=jax.ShapeDtypeStruct((s, d), A_x.dtype),
        scratch_shapes=[pltpu.VMEM((ts + _HALO, 2 * d), jnp.float32)],
        compiler_params=pltpu.CompilerParams(
            dimension_semantics=("arbitrary",),
            vmem_limit_bytes=64 * 1024 * 1024,
        ),
    )(x2, wqkv, wo, B_w1, b1, B_w2)
    return out.reshape(b, s, d)
```

```python
import functools

import jax
import jax.numpy as jnp
import jax.experimental.pallas as pl
import jax.experimental.pallas.tpu as pltpu

_H = 32
_DH = 16
_W = 8
_DIL = 2
_HALO = 16
_EPS = 1e-5


def _layernorm(x):
    m = jnp.mean(x, axis=-1, keepdims=True)
    xc = x - m
    v = jnp.mean(xc * xc, axis=-1, keepdims=True)
    return xc * jax.lax.rsqrt(v + _EPS)


def _kernel(x_ref, wqkv_ref, wo_ref, w1_ref, b1_ref, w2_ref, o_ref, kv_ref, *, ts, sub, d):
    i = pl.program_id(0)
    nchunk = d // 128

    @pl.when(i == 0)
    def _():
        kv_ref[0:_HALO, :] = jnp.zeros((_HALO, 2 * d), jnp.float32)

    @pl.when(i > 0)
    def _():
        kv_ref[0:_HALO, :] = kv_ref[ts:ts + _HALO, :]

    nsub = ts // sub

    def phase_a(r0):
        x = x_ref[r0:r0 + sub, :].astype(jnp.float32)
        xn = _layernorm(x).astype(jnp.bfloat16)
        qkv = jnp.dot(xn, wqkv_ref[...], preferred_element_type=jnp.float32)
        q = qkv[:, :d] * (_DH ** -0.5)
        kv_ref[_HALO + r0:_HALO + r0 + sub, :] = qkv[:, d:]
        row = i * ts + r0 + jax.lax.broadcasted_iota(jnp.int32, (sub, 128), 0)
        logits = []
        for w in range(_W):
            off = _HALO + r0 - w * _DIL
            acc = None
            for c in range(nchunk):
                kc = kv_ref[off:off + sub, c * 128:(c + 1) * 128]
                t = q[:, c * 128:(c + 1) * 128] * kc
                acc = t if acc is None else acc + t
            acc = acc + pltpu.roll(acc, 64, 1)
            acc = acc + pltpu.roll(acc, 32, 1)
            if w > 0:
                acc = jnp.where(row >= w * _DIL, acc, -1e9)
            logits.append(acc)
        m = functools.reduce(jnp.maximum, logits)
        ps = [jnp.exp(l - m) for l in logits]
        inv = 1.0 / functools.reduce(lambda a, b: a + b, ps)
        o_chunks = []
        for c in range(nchunk):
            acc = None
            for w in range(_W):
                off = _HALO + r0 - w * _DIL
                vc = kv_ref[off:off + sub, d + c * 128:d + (c + 1) * 128]
                t = ps[w] * vc
                acc = t if acc is None else acc + t
            o_chunks.append((acc * inv).astype(jnp.bfloat16))
        o = jnp.concatenate(o_chunks, axis=1)
        return x + jnp.dot(o, wo_ref[...], preferred_element_type=jnp.float32)

    def phase_b(r0, h):
        hn = _layernorm(h).astype(jnp.bfloat16)
        h1 = jnp.dot(hn, w1_ref[...], preferred_element_type=jnp.float32)
        h1 = h1 + b1_ref[...].astype(jnp.float32)
        e = jnp.exp(-jnp.abs(h1))
        e2 = e * e
        pos = h1 >= 0
        num = jnp.where(pos, 1.0 + 2.0 * e, e2 + 2.0 * e)
        den = num + jnp.where(pos, 2.0 * e2, 2.0)
        act = (h1 * num / den).astype(jnp.bfloat16)
        out = h + jnp.dot(act, w2_ref[...], preferred_element_type=jnp.float32)
        o_ref[r0:r0 + sub, :] = out.astype(o_ref.dtype)

    hs = []
    for j in range(nsub):
        hs.append(phase_a(j * sub))
        if j > 0:
            phase_b((j - 1) * sub, hs[j - 1])
    phase_b((nsub - 1) * sub, hs[-1])


@jax.jit
def pallas_sequential_preLN__sliding_local_dilated__dense_activation_mish__prompt_kernel(
    A_x: jax.Array,
    A_wqkv: jax.Array,
    A_wo: jax.Array,
    B_x: jax.Array,
    B_w1: jax.Array,
    B_b1: jax.Array,
    B_w2: jax.Array,
):
    b, s, d = A_x.shape
    f = B_w1.shape[1]
    ts = 512
    sub = 256
    assert b == 1 and s % ts == 0 and d == _H * _DH

    x2 = A_x.reshape(s, d)
    wqkv = A_wqkv.reshape(d, 3, _H, _DH).transpose(0, 1, 3, 2).reshape(d, 3 * d)
    wo = A_wo.reshape(_H, _DH, d).transpose(1, 0, 2).reshape(d, d)
    b1 = B_b1.reshape(1, f)

    const = lambda i: (0, 0)
    out = pl.pallas_call(
        functools.partial(_kernel, ts=ts, sub=sub, d=d),
        grid=(s // ts,),
        in_specs=[
            pl.BlockSpec((ts, d), lambda i: (i, 0)),
            pl.BlockSpec((d, 3 * d), const),
            pl.BlockSpec((d, d), const),
            pl.BlockSpec((d, f), const),
            pl.BlockSpec((1, f), const),
            pl.BlockSpec((f, d), const),
        ],
        out_specs=pl.BlockSpec((ts, d), lambda i: (i, 0)),
        out_shape=jax.ShapeDtypeStruct((s, d), A_x.dtype),
        scratch_shapes=[pltpu.VMEM((ts + _HALO, 2 * d), jnp.float32)],
        compiler_params=pltpu.CompilerParams(
            dimension_semantics=("arbitrary",),
            vmem_limit_bytes=64 * 1024 * 1024,
        ),
    )(x2, wqkv, wo, B_w1, b1, B_w2)
    return out.reshape(b, s, d)
```

```python
import functools

import jax
import jax.numpy as jnp
import jax.experimental.pallas as pl
import jax.experimental.pallas.tpu as pltpu

_H = 32
_DH = 16
_W = 8
_DIL = 2
_HALO = 16
_EPS = 1e-5
_NEG = -1e9


def _layernorm(x):
    m = jnp.mean(x, axis=-1, keepdims=True)
    xc = x - m
    v = jnp.mean(xc * xc, axis=-1, keepdims=True)
    return xc * jax.lax.rsqrt(v + _EPS)


def _kernel(x_ref, wqkv_ref, wo_ref, w1_ref, b1_ref, w2_ref, o_ref,
            q_ref, kv_ref, a_ref, h_ref, *, ts, d, f, nt):
    i = pl.program_id(0)
    nchunk = d // 128
    rb = 32
    nrb = ts // rb
    fch = 128
    nf = -(-f // fch)

    def qkv_stage():
        x = x_ref[...].astype(jnp.float32)
        xn = _layernorm(x).astype(jnp.bfloat16)
        qkv = jnp.dot(xn, wqkv_ref[...], preferred_element_type=jnp.float32)
        q_ref[...] = qkv[:, :d] * (_DH ** -0.5)
        kv_ref[_HALO:_HALO + ts, :] = qkv[:, d:]

    def attn_block(r0, masked):
        logits = []
        for w in range(_W):
            off = _HALO + r0 - w * _DIL
            acc = None
            for c in range(nchunk):
                kc = kv_ref[off:off + rb, c * 128:(c + 1) * 128]
                t = q_ref[r0:r0 + rb, c * 128:(c + 1) * 128] * kc
                acc = t if acc is None else acc + t
            acc = acc + pltpu.roll(acc, 64, 1)
            acc = acc + pltpu.roll(acc, 32, 1)
            if masked and w > 0 and r0 < w * _DIL:
                row = r0 + jax.lax.broadcasted_iota(jnp.int32, (rb, 128), 0)
                acc = jnp.where(row >= w * _DIL, acc, _NEG)
            logits.append(acc)
        m = functools.reduce(jnp.maximum, logits)
        ps = [jnp.exp(l - m) for l in logits]
        inv = 1.0 / functools.reduce(lambda a, b: a + b, ps)
        for c in range(nchunk):
            acc = None
            for w in range(_W):
                off = _HALO + r0 - w * _DIL
                vc = kv_ref[off:off + rb, d + c * 128:d + (c + 1) * 128]
                t = ps[w] * vc
                acc = t if acc is None else acc + t
            a_ref[r0:r0 + rb, c * 128:(c + 1) * 128] = (acc * inv).astype(jnp.bfloat16)

    def wo_stage():
        x = x_ref[...].astype(jnp.float32)
        h_ref[...] = x + jnp.dot(a_ref[...], wo_ref[...],
                                 preferred_element_type=jnp.float32)

    def mlp_chunk(hn, j, acc):
        lo = j * fch
        hi = min(f, lo + fch)
        h1 = jnp.dot(hn, w1_ref[:, lo:hi], preferred_element_type=jnp.float32)
        h1 = h1 + b1_ref[:, lo:hi].astype(jnp.float32)
        e = jnp.exp(-jnp.abs(h1))
        e2 = e * e
        pos = h1 >= 0
        num = jnp.where(pos, 1.0 + 2.0 * e, e2 + 2.0 * e)
        den = num + jnp.where(pos, 2.0 * e2, 2.0)
        act = (h1 * num / den).astype(jnp.bfloat16)
        y = jnp.dot(act, w2_ref[lo:hi, :], preferred_element_type=jnp.float32)
        return y if acc is None else acc + y

    def run(do_a, do_b, masked):
        if do_b:
            h = h_ref[...]
            hn = _layernorm(h).astype(jnp.bfloat16)
        if do_a:
            qkv_stage()
        acc = None
        for j in range(max(nf, nrb)):
            if do_b and j < nf:
                acc = mlp_chunk(hn, j, acc if acc is not None else h)
            if do_a and j < nrb:
                attn_block(j * rb, masked)
        if do_b:
            o_ref[...] = acc.astype(o_ref.dtype)
        if do_a:
            wo_stage()

    @pl.when(i == 0)
    def _():
        kv_ref[0:_HALO, :] = jnp.zeros((_HALO, 2 * d), jnp.float32)
        run(True, False, True)

    @pl.when((i > 0) & (i < nt))
    def _():
        kv_ref[0:_HALO, :] = kv_ref[ts:ts + _HALO, :]
        run(True, True, False)

    @pl.when(i == nt)
    def _():
        run(False, True, False)


@jax.jit
def pallas_sequential_preLN__sliding_local_dilated__dense_activation_mish__prompt_kernel(
    A_x: jax.Array,
    A_wqkv: jax.Array,
    A_wo: jax.Array,
    B_x: jax.Array,
    B_w1: jax.Array,
    B_b1: jax.Array,
    B_w2: jax.Array,
):
    b, s, d = A_x.shape
    f = B_w1.shape[1]
    ts = 256
    nt = s // ts
    assert b == 1 and s % ts == 0 and d == _H * _DH

    x2 = A_x.reshape(s, d)
    wqkv = A_wqkv.reshape(d, 3, _H, _DH).transpose(0, 1, 3, 2).reshape(d, 3 * d)
    wo = A_wo.reshape(_H, _DH, d).transpose(1, 0, 2).reshape(d, d)
    b1 = B_b1.reshape(1, f)

    const = lambda i: (0, 0)
    out = pl.pallas_call(
        functools.partial(_kernel, ts=ts, d=d, f=f, nt=nt),
        grid=(nt + 1,),
        in_specs=[
            pl.BlockSpec((ts, d), lambda i: (jnp.minimum(i, nt - 1), 0)),
            pl.BlockSpec((d, 3 * d), const),
            pl.BlockSpec((d, d), const),
            pl.BlockSpec((d, f), const),
            pl.BlockSpec((1, f), const),
            pl.BlockSpec((f, d), const),
        ],
        out_specs=pl.BlockSpec((ts, d), lambda i: (jnp.maximum(i - 1, 0), 0)),
        out_shape=jax.ShapeDtypeStruct((s, d), A_x.dtype),
        scratch_shapes=[
            pltpu.VMEM((ts, d), jnp.float32),
            pltpu.VMEM((ts + _HALO, 2 * d), jnp.float32),
            pltpu.VMEM((ts, d), jnp.bfloat16),
            pltpu.VMEM((ts, d), jnp.float32),
        ],
        compiler_params=pltpu.CompilerParams(
            dimension_semantics=("arbitrary",),
            vmem_limit_bytes=64 * 1024 * 1024,
        ),
    )(x2, wqkv, wo, B_w1, b1, B_w2)
    return out.reshape(b, s, d)
```

```python
import functools

import jax
import jax.numpy as jnp
import jax.experimental.pallas as pl
import jax.experimental.pallas.tpu as pltpu

_H = 32
_DH = 16
_W = 8
_DIL = 2
_HALO = 16
_EPS = 1e-5
_NEG = -1e9


def _layernorm(x):
    m = jnp.mean(x, axis=-1, keepdims=True)
    xc = x - m
    v = jnp.mean(xc * xc, axis=-1, keepdims=True)
    return xc * jax.lax.rsqrt(v + _EPS)


def _kernel(x_ref, xp_ref, wqkv_ref, wo_ref, w1_ref, b1_ref, w2_ref, o_ref,
            q_ref, kv_ref, a_ref, *, ts, d, f, nt):
    i = pl.program_id(0)
    nchunk = d // 128
    rb = 32
    nrb = ts // rb
    fch = 128
    nf = -(-f // fch)

    def qkv_stage():
        x = x_ref[...].astype(jnp.float32)
        xn = _layernorm(x).astype(jnp.bfloat16)
        qkv = jnp.dot(xn, wqkv_ref[...], preferred_element_type=jnp.float32)
        q_ref[...] = qkv[:, :d] * (_DH ** -0.5)
        kv_ref[_HALO:_HALO + ts, :] = qkv[:, d:]

    def attn_block(r0, masked):
        logits = []
        for w in range(_W):
            off = _HALO + r0 - w * _DIL
            acc = None
            for c in range(nchunk):
                kc = kv_ref[off:off + rb, c * 128:(c + 1) * 128]
                t = q_ref[r0:r0 + rb, c * 128:(c + 1) * 128] * kc
                acc = t if acc is None else acc + t
            acc = acc + pltpu.roll(acc, 64, 1)
            acc = acc + pltpu.roll(acc, 32, 1)
            if masked and w > 0 and r0 < w * _DIL:
                row = r0 + jax.lax.broadcasted_iota(jnp.int32, (rb, 128), 0)
                acc = jnp.where(row >= w * _DIL, acc, _NEG)
            logits.append(acc)
        m = functools.reduce(jnp.maximum, logits)
        ps = [jnp.exp(l - m) for l in logits]
        inv = 1.0 / functools.reduce(lambda a, b: a + b, ps)
        for c in range(nchunk):
            acc = None
            for w in range(_W):
                off = _HALO + r0 - w * _DIL
                vc = kv_ref[off:off + rb, d + c * 128:d + (c + 1) * 128]
                t = ps[w] * vc
                acc = t if acc is None else acc + t
            a_ref[r0:r0 + rb, c * 128:(c + 1) * 128] = (acc * inv).astype(jnp.bfloat16)

    def wo_stage():
        x = xp_ref[...].astype(jnp.float32)
        return x + jnp.dot(a_ref[...], wo_ref[...],
                           preferred_element_type=jnp.float32)

    def mlp_chunk(hn, j, acc):
        lo = j * fch
        hi = min(f, lo + fch)
        h1 = jnp.dot(hn, w1_ref[:, lo:hi], preferred_element_type=jnp.float32)
        h1 = h1 + b1_ref[:, lo:hi].astype(jnp.float32)
        e = jnp.exp(-jnp.abs(h1))
        e2 = e * e
        pos = h1 >= 0
        num = jnp.where(pos, 1.0 + 2.0 * e, e2 + 2.0 * e)
        den = num + jnp.where(pos, 2.0 * e2, 2.0)
        act = (h1 * num / den).astype(jnp.bfloat16)
        y = jnp.dot(act, w2_ref[lo:hi, :], preferred_element_type=jnp.float32)
        return y if acc is None else acc + y

    def run(do_a, do_b, masked):
        if do_b:
            h = wo_stage()
            hn = _layernorm(h).astype(jnp.bfloat16)
        if do_a:
            qkv_stage()
        acc = None
        for j in range(max(nf, nrb)):
            if do_b and j < nf:
                acc = mlp_chunk(hn, j, acc if acc is not None else h)
            if do_a and j < nrb:
                attn_block(j * rb, masked)
        if do_b:
            o_ref[...] = acc.astype(o_ref.dtype)

    @pl.when(i == 0)
    def _():
        kv_ref[0:_HALO, :] = jnp.zeros((_HALO, 2 * d), jnp.float32)
        run(True, False, True)

    @pl.when((i > 0) & (i < nt))
    def _():
        kv_ref[0:_HALO, :] = kv_ref[ts:ts + _HALO, :]
        run(True, True, False)

    @pl.when(i == nt)
    def _():
        run(False, True, False)


@jax.jit
def pallas_sequential_preLN__sliding_local_dilated__dense_activation_mish__prompt_kernel(
    A_x: jax.Array,
    A_wqkv: jax.Array,
    A_wo: jax.Array,
    B_x: jax.Array,
    B_w1: jax.Array,
    B_b1: jax.Array,
    B_w2: jax.Array,
):
    b, s, d = A_x.shape
    f = B_w1.shape[1]
    ts = 256
    nt = s // ts
    assert b == 1 and s % ts == 0 and d == _H * _DH

    x2 = A_x.reshape(s, d)
    wqkv = A_wqkv.reshape(d, 3, _H, _DH).transpose(0, 1, 3, 2).reshape(d, 3 * d)
    wo = A_wo.reshape(_H, _DH, d).transpose(1, 0, 2).reshape(d, d)
    b1 = B_b1.reshape(1, f)

    const = lambda i: (0, 0)
    out = pl.pallas_call(
        functools.partial(_kernel, ts=ts, d=d, f=f, nt=nt),
        grid=(nt + 1,),
        in_specs=[
            pl.BlockSpec((ts, d), lambda i: (jnp.minimum(i, nt - 1), 0)),
            pl.BlockSpec((ts, d), lambda i: (jnp.maximum(i - 1, 0), 0)),
            pl.BlockSpec((d, 3 * d), const),
            pl.BlockSpec((d, d), const),
            pl.BlockSpec((d, f), const),
            pl.BlockSpec((1, f), const),
            pl.BlockSpec((f, d), const),
        ],
        out_specs=pl.BlockSpec((ts, d), lambda i: (jnp.maximum(i - 1, 0), 0)),
        out_shape=jax.ShapeDtypeStruct((s, d), A_x.dtype),
        scratch_shapes=[
            pltpu.VMEM((ts, d), jnp.float32),
            pltpu.VMEM((ts + _HALO, 2 * d), jnp.float32),
            pltpu.VMEM((ts, d), jnp.bfloat16),
        ],
        compiler_params=pltpu.CompilerParams(
            dimension_semantics=("arbitrary",),
            vmem_limit_bytes=64 * 1024 * 1024,
        ),
    )(x2, x2, wqkv, wo, B_w1, b1, B_w2)
    return out.reshape(b, s, d)
```

```python
import functools

import jax
import jax.numpy as jnp
import jax.experimental.pallas as pl
import jax.experimental.pallas.tpu as pltpu

_H = 32
_DH = 16
_W = 8
_DIL = 2
_HALO = 16
_EPS = 1e-5
_NEG = -1e9


def _layernorm(x):
    m = jnp.mean(x, axis=-1, keepdims=True)
    xc = x - m
    v = jnp.mean(xc * xc, axis=-1, keepdims=True)
    return xc * jax.lax.rsqrt(v + _EPS)


def _kernel(x_ref, xp_ref, wqkv_ref, wo_ref, w1_ref, b1_ref, w2_ref, o_ref,
            q_ref, kv_ref, a_ref, hn_ref, acc_ref, st_ref, *, ts, d, f, nt):
    i = pl.program_id(0)
    nchunk = d // 128
    rb = 32
    nrb = ts // rb
    fch = 128
    nf = -(-f // fch)

    def qkv_stage():
        x = x_ref[...].astype(jnp.float32)
        xn = _layernorm(x).astype(jnp.bfloat16)
        qkv = jnp.dot(xn, wqkv_ref[...], preferred_element_type=jnp.float32)
        q_ref[...] = qkv[:, :d] * (_DH ** -0.5)
        kv_ref[_HALO:_HALO + ts, :] = qkv[:, d:]

    def attn_block(r0, masked):
        st_ref[...] = kv_ref[pl.ds(r0, rb + _HALO), :]
        logits = []
        for w in range(_W):
            off = _HALO - w * _DIL
            acc = None
            for c in range(nchunk):
                kc = st_ref[off:off + rb, c * 128:(c + 1) * 128]
                t = q_ref[pl.ds(r0, rb), c * 128:(c + 1) * 128] * kc
                acc = t if acc is None else acc + t
            acc = acc + pltpu.roll(acc, 64, 1)
            acc = acc + pltpu.roll(acc, 32, 1)
            if masked and w > 0:
                row = r0 + jax.lax.broadcasted_iota(jnp.int32, (rb, 128), 0)
                acc = jnp.where(row >= w * _DIL, acc, _NEG)
            logits.append(acc)
        m = functools.reduce(jnp.maximum, logits)
        ps = [jnp.exp(l - m) for l in logits]
        inv = 1.0 / functools.reduce(lambda a, b: a + b, ps)
        for c in range(nchunk):
            acc = None
            for w in range(_W):
                off = _HALO - w * _DIL
                vc = st_ref[off:off + rb, d + c * 128:d + (c + 1) * 128]
                t = ps[w] * vc
                acc = t if acc is None else acc + t
            a_ref[pl.ds(r0, rb), c * 128:(c + 1) * 128] = (acc * inv).astype(jnp.bfloat16)

    def wo_stage():
        x = xp_ref[...].astype(jnp.float32)
        return x + jnp.dot(a_ref[...], wo_ref[...],
                           preferred_element_type=jnp.float32)

    def mlp_chunk(lo, width):
        h1 = jnp.dot(hn_ref[...], w1_ref[:, pl.ds(lo, width)],
                     preferred_element_type=jnp.float32)
        h1 = h1 + b1_ref[:, pl.ds(lo, width)].astype(jnp.float32)
        e = jnp.exp(-jnp.abs(h1))
        e2 = e * e
        pos = h1 >= 0
        num = jnp.where(pos, 1.0 + 2.0 * e, e2 + 2.0 * e)
        den = num + jnp.where(pos, 2.0 * e2, 2.0)
        act = (h1 * num / den).astype(jnp.bfloat16)
        acc_ref[...] += jnp.dot(act, w2_ref[pl.ds(lo, width), :],
                                preferred_element_type=jnp.float32)

    def run(do_a, do_b, masked):
        if do_b:
            h = wo_stage()
            acc_ref[...] = h
            hn_ref[...] = _layernorm(h).astype(jnp.bfloat16)
            for j in range(nrb, nf):
                mlp_chunk(j * fch, min(fch, f - j * fch))
        if do_a:
            qkv_stage()

        def body(j, carry):
            if do_b:
                mlp_chunk(pl.multiple_of(j * fch, fch), fch)
            if do_a:
                attn_block(pl.multiple_of(j * rb, rb), masked)
            return carry

        jax.lax.fori_loop(0, nrb, body, 0)
        if do_b:
            o_ref[...] = acc_ref[...].astype(o_ref.dtype)

    @pl.when(i == 0)
    def _():
        kv_ref[0:_HALO, :] = jnp.zeros((_HALO, 2 * d), jnp.float32)
        run(True, False, True)

    @pl.when((i > 0) & (i < nt))
    def _():
        kv_ref[0:_HALO, :] = kv_ref[ts:ts + _HALO, :]
        run(True, True, False)

    @pl.when(i == nt)
    def _():
        run(False, True, False)


@jax.jit
def pallas_sequential_preLN__sliding_local_dilated__dense_activation_mish__prompt_kernel(
    A_x: jax.Array,
    A_wqkv: jax.Array,
    A_wo: jax.Array,
    B_x: jax.Array,
    B_w1: jax.Array,
    B_b1: jax.Array,
    B_w2: jax.Array,
):
    b, s, d = A_x.shape
    f = B_w1.shape[1]
    ts = 256
    nt = s // ts
    assert b == 1 and s % ts == 0 and d == _H * _DH

    x2 = A_x.reshape(s, d)
    wqkv = A_wqkv.reshape(d, 3, _H, _DH).transpose(0, 1, 3, 2).reshape(d, 3 * d)
    wo = A_wo.reshape(_H, _DH, d).transpose(1, 0, 2).reshape(d, d)
    b1 = B_b1.reshape(1, f)

    const = lambda i: (0, 0)
    out = pl.pallas_call(
        functools.partial(_kernel, ts=ts, d=d, f=f, nt=nt),
        grid=(nt + 1,),
        in_specs=[
            pl.BlockSpec((ts, d), lambda i: (jnp.minimum(i, nt - 1), 0)),
            pl.BlockSpec((ts, d), lambda i: (jnp.maximum(i - 1, 0), 0)),
            pl.BlockSpec((d, 3 * d), const),
            pl.BlockSpec((d, d), const),
            pl.BlockSpec((d, f), const),
            pl.BlockSpec((1, f), const),
            pl.BlockSpec((f, d), const),
        ],
        out_specs=pl.BlockSpec((ts, d), lambda i: (jnp.maximum(i - 1, 0), 0)),
        out_shape=jax.ShapeDtypeStruct((s, d), A_x.dtype),
        scratch_shapes=[
            pltpu.VMEM((ts, d), jnp.float32),
            pltpu.VMEM((ts + _HALO, 2 * d), jnp.float32),
            pltpu.VMEM((ts, d), jnp.bfloat16),
            pltpu.VMEM((ts, d), jnp.bfloat16),
            pltpu.VMEM((ts, d), jnp.float32),
            pltpu.VMEM((32 + _HALO, 2 * d), jnp.float32),
        ],
        compiler_params=pltpu.CompilerParams(
            dimension_semantics=("arbitrary",),
            vmem_limit_bytes=64 * 1024 * 1024,
        ),
    )(x2, x2, wqkv, wo, B_w1, b1, B_w2)
    return out.reshape(b, s, d)
```

```python
import functools

import jax
import jax.numpy as jnp
import jax.experimental.pallas as pl
import jax.experimental.pallas.tpu as pltpu

_H = 32
_DH = 16
_W = 8
_DIL = 2
_HALO = 16
_EPS = 1e-5
_NEG = -1e9


def _layernorm(x):
    m = jnp.mean(x, axis=-1, keepdims=True)
    xc = x - m
    v = jnp.mean(xc * xc, axis=-1, keepdims=True)
    return xc * jax.lax.rsqrt(v + _EPS)


def _kernel(x_ref, xp_ref, wqkv_ref, wo_in_ref, w1_ref, b1_ref, w2_ref, o_ref,
            wp_ref, wo_ref, q_ref, kv_ref, a_ref, *, ts, d, f, nt):
    i = pl.program_id(0)
    nchunk = d // 128
    rb = 32
    nrb = ts // rb
    fch = 128
    nf = -(-f // fch)

    def permute_weights():
        r = jax.lax.broadcasted_iota(jnp.int32, (d, d), 0)
        c = jax.lax.broadcasted_iota(jnp.int32, (d, d), 1)
        perm = (c == (r % _DH) * _H + r // _DH).astype(jnp.bfloat16)
        perm_t = (r == (c % _DH) * _H + c // _DH).astype(jnp.bfloat16)
        wo_ref[...] = jnp.dot(perm_t, wo_in_ref[...],
                              preferred_element_type=jnp.float32).astype(jnp.bfloat16)
        for t in range(3):
            wp_ref[:, t * d:(t + 1) * d] = jnp.dot(
                wqkv_ref[:, t * d:(t + 1) * d], perm,
                preferred_element_type=jnp.float32).astype(jnp.bfloat16)

    def qkv_stage():
        x = x_ref[...].astype(jnp.float32)
        xn = _layernorm(x).astype(jnp.bfloat16)
        qkv = jnp.dot(xn, wp_ref[...], preferred_element_type=jnp.float32)
        q_ref[...] = qkv[:, :d] * (_DH ** -0.5)
        kv_ref[_HALO:_HALO + ts, :] = qkv[:, d:]

    def attn_block(r0, masked):
        logits = []
        for w in range(_W):
            off = _HALO + r0 - w * _DIL
            acc = None
            for c in range(nchunk):
                kc = kv_ref[off:off + rb, c * 128:(c + 1) * 128]
                t = q_ref[r0:r0 + rb, c * 128:(c + 1) * 128] * kc
                acc = t if acc is None else acc + t
            acc = acc + pltpu.roll(acc, 64, 1)
            acc = acc + pltpu.roll(acc, 32, 1)
            if masked and w > 0 and r0 < w * _DIL:
                row = r0 + jax.lax.broadcasted_iota(jnp.int32, (rb, 128), 0)
                acc = jnp.where(row >= w * _DIL, acc, _NEG)
            logits.append(acc)
        m = functools.reduce(jnp.maximum, logits)
        ps = [jnp.exp(l - m) for l in logits]
        inv = 1.0 / functools.reduce(lambda a, b: a + b, ps)
        for c in range(nchunk):
            acc = None
            for w in range(_W):
                off = _HALO + r0 - w * _DIL
                vc = kv_ref[off:off + rb, d + c * 128:d + (c + 1) * 128]
                t = ps[w] * vc
                acc = t if acc is None else acc + t
            a_ref[r0:r0 + rb, c * 128:(c + 1) * 128] = (acc * inv).astype(jnp.bfloat16)

    def wo_stage():
        x = xp_ref[...].astype(jnp.float32)
        return x + jnp.dot(a_ref[...], wo_ref[...],
                           preferred_element_type=jnp.float32)

    def mlp_chunk(hn, j, acc):
        lo = j * fch
        hi = min(f, lo + fch)
        h1 = jax.lax.dot_general(hn, w1_ref[lo:hi, :], (((1,), (1,)), ((), ())),
                                 preferred_element_type=jnp.float32)
        h1 = h1 + b1_ref[:, lo:hi].astype(jnp.float32)
        e = jnp.exp(-jnp.abs(h1))
        e2 = e * e
        pos = h1 >= 0
        num = jnp.where(pos, 1.0 + 2.0 * e, e2 + 2.0 * e)
        den = num + jnp.where(pos, 2.0 * e2, 2.0)
        act = (h1 * num / den).astype(jnp.bfloat16)
        y = jnp.dot(act, w2_ref[lo:hi, :], preferred_element_type=jnp.float32)
        return acc + y

    def run(do_a, do_b, masked):
        if do_b:
            h = wo_stage()
            hn = _layernorm(h).astype(jnp.bfloat16)
        if do_a:
            qkv_stage()
        acc = h if do_b else None
        for j in range(max(nf, nrb)):
            if do_b and j < nf:
                acc = mlp_chunk(hn, j, acc)
            if do_a and j < nrb:
                attn_block(j * rb, masked)
        if do_b:
            o_ref[...] = acc.astype(o_ref.dtype)

    @pl.when(i == 0)
    def _():
        permute_weights()
        kv_ref[0:_HALO, :] = jnp.zeros((_HALO, 2 * d), jnp.float32)
        run(True, False, True)

    @pl.when((i > 0) & (i < nt))
    def _():
        kv_ref[0:_HALO, :] = kv_ref[ts:ts + _HALO, :]
        run(True, True, False)

    @pl.when(i == nt)
    def _():
        run(False, True, False)


@jax.jit
def pallas_sequential_preLN__sliding_local_dilated__dense_activation_mish__prompt_kernel(
    A_x: jax.Array,
    A_wqkv: jax.Array,
    A_wo: jax.Array,
    B_x: jax.Array,
    B_w1: jax.Array,
    B_b1: jax.Array,
    B_w2: jax.Array,
):
    b, s, d = A_x.shape
    f = B_w1.shape[1]
    ts = 256
    nt = s // ts
    assert b == 1 and s % ts == 0 and d == _H * _DH

    x2 = A_x.reshape(s, d)
    b1 = B_b1.reshape(1, f)

    const = lambda i: (0, 0)
    out = pl.pallas_call(
        functools.partial(_kernel, ts=ts, d=d, f=f, nt=nt),
        grid=(nt + 1,),
        in_specs=[
            pl.BlockSpec((ts, d), lambda i: (jnp.minimum(i, nt - 1), 0)),
            pl.BlockSpec((ts, d), lambda i: (jnp.maximum(i - 1, 0), 0)),
            pl.BlockSpec((d, 3 * d), const),
            pl.BlockSpec((d, d), const),
            pl.BlockSpec((f, d), const),
            pl.BlockSpec((1, f), const),
            pl.BlockSpec((f, d), const),
        ],
        out_specs=pl.BlockSpec((ts, d), lambda i: (jnp.maximum(i - 1, 0), 0)),
        out_shape=jax.ShapeDtypeStruct((s, d), A_x.dtype),
        scratch_shapes=[
            pltpu.VMEM((d, 3 * d), jnp.bfloat16),
            pltpu.VMEM((d, d), jnp.bfloat16),
            pltpu.VMEM((ts, d), jnp.float32),
            pltpu.VMEM((ts + _HALO, 2 * d), jnp.float32),
            pltpu.VMEM((ts, d), jnp.bfloat16),
        ],
        compiler_params=pltpu.CompilerParams(
            dimension_semantics=("arbitrary",),
            vmem_limit_bytes=64 * 1024 * 1024,
        ),
    )(x2, x2, A_wqkv, A_wo, B_w1.T, b1, B_w2)
    return out.reshape(b, s, d)
```

```python
import functools

import jax
import jax.numpy as jnp
import jax.experimental.pallas as pl
import jax.experimental.pallas.tpu as pltpu

_H = 32
_DH = 16
_W = 8
_DIL = 2
_HALO = 16
_EPS = 1e-5
_NEG = -1e9


def _layernorm(x):
    m = jnp.mean(x, axis=-1, keepdims=True)
    xc = x - m
    v = jnp.mean(xc * xc, axis=-1, keepdims=True)
    return xc * jax.lax.rsqrt(v + _EPS)


def _kernel(x_ref, xp_ref, wqkv_ref, wo_in_ref, w1_ref, b1_ref, w2_ref, o_ref,
            wp_ref, wo_ref, xn_ref, qkv_ref, st_ref, a_ref, *, ts, d, f, nt):
    i = pl.program_id(0)
    nchunk = d // 128
    nj = 4
    rb = ts // nj
    nc = 3 * d // nj
    fch = 128
    nf = -(-f // fch)
    cur = i % 2
    prv = 1 - cur

    def permute_weights():
        r = jax.lax.broadcasted_iota(jnp.int32, (d, d), 0)
        c = jax.lax.broadcasted_iota(jnp.int32, (d, d), 1)
        perm = (c == (r % _DH) * _H + r // _DH).astype(jnp.bfloat16)
        perm_t = (r == (c % _DH) * _H + c // _DH).astype(jnp.bfloat16)
        wo_ref[...] = jnp.dot(perm_t, wo_in_ref[...],
                              preferred_element_type=jnp.float32).astype(jnp.bfloat16)
        for t in range(3):
            wt = jnp.dot(wqkv_ref[:, t * d:(t + 1) * d], perm,
                         preferred_element_type=jnp.float32)
            if t == 0:
                wt = wt * (_DH ** -0.5)
            wp_ref[:, t * d:(t + 1) * d] = wt.astype(jnp.bfloat16)

    def ln1_stage():
        x = x_ref[...].astype(jnp.float32)
        xn_ref[...] = _layernorm(x).astype(jnp.bfloat16)

    def qkv_chunk(c0):
        qkv_ref[cur, _HALO:_HALO + ts, pl.ds(c0, nc)] = jnp.dot(
            xn_ref[...], wp_ref[:, pl.ds(c0, nc)], preferred_element_type=jnp.float32)

    def attn_block(r0, masked):
        st_ref[...] = qkv_ref[prv, pl.ds(r0, rb + _HALO), d:]
        logits = []
        for w in range(_W):
            off = _HALO - w * _DIL
            acc = None
            for c in range(nchunk):
                kc = st_ref[off:off + rb, c * 128:(c + 1) * 128]
                qc = qkv_ref[prv, pl.ds(r0 + _HALO, rb), c * 128:(c + 1) * 128]
                t = qc * kc
                acc = t if acc is None else acc + t
            acc = acc + pltpu.roll(acc, 64, 1)
            acc = acc + pltpu.roll(acc, 32, 1)
            if masked and w > 0:
                row = r0 + jax.lax.broadcasted_iota(jnp.int32, (rb, 128), 0)
                acc = jnp.where(row >= w * _DIL, acc, _NEG)
            logits.append(acc)
        m = functools.reduce(jnp.maximum, logits)
        ps = [jnp.exp(l - m) for l in logits]
        inv = 1.0 / functools.reduce(lambda a, b: a + b, ps)
        for c in range(nchunk):
            acc = None
            for w in range(_W):
                off = _HALO - w * _DIL
                vc = st_ref[off:off + rb, d + c * 128:d + (c + 1) * 128]
                t = ps[w] * vc
                acc = t if acc is None else acc + t
            a_ref[pl.ds(r0, rb), c * 128:(c + 1) * 128] = (acc * inv).astype(jnp.bfloat16)

    def mlp_chunk(hn, j, acc):
        lo = j * fch
        hi = min(f, lo + fch)
        h1 = jax.lax.dot_general(hn, w1_ref[lo:hi, :], (((1,), (1,)), ((), ())),
                                 preferred_element_type=jnp.float32)
        h1 = h1 + b1_ref[:, lo:hi].astype(jnp.float32)
        e = jnp.exp(-jnp.abs(h1))
        e2 = e * e
        pos = h1 >= 0
        num = jnp.where(pos, 1.0 + 2.0 * e, e2 + 2.0 * e)
        den = num + jnp.where(pos, 2.0 * e2, 2.0)
        act = (h1 * num / den).astype(jnp.bfloat16)
        y = jnp.dot(act, w2_ref[lo:hi, :], preferred_element_type=jnp.float32)
        return acc + y

    def run(do_a, do_b, masked):
        if do_a:
            ln1_stage()

        def body(j, carry):
            if do_a:
                qkv_chunk(pl.multiple_of(j * nc, 128))
            if do_b:
                attn_block(pl.multiple_of(j * rb, rb), masked)
            return carry

        jax.lax.fori_loop(0, nj, body, 0)
        if do_b:
            x = xp_ref[...].astype(jnp.float32)
            h = x + jnp.dot(a_ref[...], wo_ref[...], preferred_element_type=jnp.float32)
            hn = _layernorm(h).astype(jnp.bfloat16)
            acc = h
            for j in range(nf):
                acc = mlp_chunk(hn, j, acc)
            o_ref[...] = acc.astype(o_ref.dtype)

    def carry_halo():
        qkv_ref[cur, 0:_HALO, d:] = qkv_ref[prv, ts:ts + _HALO, d:]

    @pl.when(i == 0)
    def _():
        permute_weights()
        qkv_ref[0, 0:_HALO, d:] = jnp.zeros((_HALO, 2 * d), jnp.float32)
        run(True, False, False)

    @pl.when(i == 1)
    def _():
        carry_halo()
        run(True, True, True)

    @pl.when((i > 1) & (i < nt))
    def _():
        carry_halo()
        run(True, True, False)

    @pl.when(i == nt)
    def _():
        run(False, True, False)


@jax.jit
def pallas_sequential_preLN__sliding_local_dilated__dense_activation_mish__prompt_kernel(
    A_x: jax.Array,
    A_wqkv: jax.Array,
    A_wo: jax.Array,
    B_x: jax.Array,
    B_w1: jax.Array,
    B_b1: jax.Array,
    B_w2: jax.Array,
):
    b, s, d = A_x.shape
    f = B_w1.shape[1]
    ts = 256
    nt = s // ts
    assert b == 1 and s % ts == 0 and d == _H * _DH

    x2 = A_x.reshape(s, d)
    b1 = B_b1.reshape(1, f)

    const = lambda i: (0, 0)
    out = pl.pallas_call(
        functools.partial(_kernel, ts=ts, d=d, f=f, nt=nt),
        grid=(nt + 1,),
        in_specs=[
            pl.BlockSpec((ts, d), lambda i: (jnp.minimum(i, nt - 1), 0)),
            pl.BlockSpec((ts, d), lambda i: (jnp.maximum(i - 1, 0), 0)),
            pl.BlockSpec((d, 3 * d), const),
            pl.BlockSpec((d, d), const),
            pl.BlockSpec((f, d), const),
            pl.BlockSpec((1, f), const),
            pl.BlockSpec((f, d), const),
        ],
        out_specs=pl.BlockSpec((ts, d), lambda i: (jnp.maximum(i - 1, 0), 0)),
        out_shape=jax.ShapeDtypeStruct((s, d), A_x.dtype),
        scratch_shapes=[
            pltpu.VMEM((d, 3 * d), jnp.bfloat16),
            pltpu.VMEM((d, d), jnp.bfloat16),
            pltpu.VMEM((ts, d), jnp.bfloat16),
            pltpu.VMEM((2, ts + _HALO, 3 * d), jnp.float32),
            pltpu.VMEM((ts // 4 + _HALO, 2 * d), jnp.float32),
            pltpu.VMEM((ts, d), jnp.bfloat16),
        ],
        compiler_params=pltpu.CompilerParams(
            dimension_semantics=("arbitrary",),
            vmem_limit_bytes=64 * 1024 * 1024,
        ),
    )(x2, x2, A_wqkv, A_wo, B_w1.T, b1, B_w2)
    return out.reshape(b, s, d)
```

```python
import functools

import jax
import jax.numpy as jnp
import jax.experimental.pallas as pl
import jax.experimental.pallas.tpu as pltpu

_H = 32
_DH = 16
_W = 8
_DIL = 2
_HALO = 16
_EPS = 1e-5
_NEG = -1e9


def _layernorm(x):
    m = jnp.mean(x, axis=-1, keepdims=True)
    xc = x - m
    v = jnp.mean(xc * xc, axis=-1, keepdims=True)
    return xc * jax.lax.rsqrt(v + _EPS)


def _kernel(x_ref, xp_ref, wqkv_ref, wo_in_ref, w1_ref, b1_ref, w2_ref, o_ref,
            wp_ref, wo_ref, xn_ref, qkv0_ref, qkv1_ref, st_ref, a_ref, *, ts, d, f, nt):
    i = pl.program_id(0)
    nchunk = d // 128
    nj = 4
    rb = ts // nj
    nc = 3 * d // nj
    fch = 128
    nf = -(-f // fch)
    bufs = (qkv0_ref, qkv1_ref)

    def permute_weights():
        r = jax.lax.broadcasted_iota(jnp.int32, (d, d), 0)
        c = jax.lax.broadcasted_iota(jnp.int32, (d, d), 1)
        perm = (c == (r % _DH) * _H + r // _DH).astype(jnp.bfloat16)
        perm_t = (r == (c % _DH) * _H + c // _DH).astype(jnp.bfloat16)
        wo_ref[...] = jnp.dot(perm_t, wo_in_ref[...],
                              preferred_element_type=jnp.float32).astype(jnp.bfloat16)
        for t in range(3):
            wt = jnp.dot(wqkv_ref[:, t * d:(t + 1) * d], perm,
                         preferred_element_type=jnp.float32)
            if t == 0:
                wt = wt * (_DH ** -0.5)
            wp_ref[:, t * d:(t + 1) * d] = wt.astype(jnp.bfloat16)

    def ln1_stage():
        x = x_ref[...].astype(jnp.float32)
        xn_ref[...] = _layernorm(x).astype(jnp.bfloat16)

    def qkv_chunk(wr_ref, c0):
        wr_ref[_HALO:_HALO + ts, pl.ds(c0, nc)] = jnp.dot(
            xn_ref[...], wp_ref[:, pl.ds(c0, nc)], preferred_element_type=jnp.float32)

    def attn_block(rd_ref, r0, masked):
        st_ref[...] = rd_ref[pl.ds(r0, rb + _HALO), d:]
        logits = []
        for w in range(_W):
            off = _HALO - w * _DIL
            acc = None
            for c in range(nchunk):
                kc = st_ref[off:off + rb, c * 128:(c + 1) * 128]
                qc = rd_ref[pl.ds(r0 + _HALO, rb), c * 128:(c + 1) * 128]
                t = qc * kc
                acc = t if acc is None else acc + t
            acc = acc + pltpu.roll(acc, 64, 1)
            acc = acc + pltpu.roll(acc, 32, 1)
            if masked and w > 0:
                row = r0 + jax.lax.broadcasted_iota(jnp.int32, (rb, 128), 0)
                acc = jnp.where(row >= w * _DIL, acc, _NEG)
            logits.append(acc)
        m = functools.reduce(jnp.maximum, logits)
        ps = [jnp.exp(l - m) for l in logits]
        inv = 1.0 / functools.reduce(lambda a, b: a + b, ps)
        for c in range(nchunk):
            acc = None
            for w in range(_W):
                off = _HALO - w * _DIL
                vc = st_ref[off:off + rb, d + c * 128:d + (c + 1) * 128]
                t = ps[w] * vc
                acc = t if acc is None else acc + t
            a_ref[pl.ds(r0, rb), c * 128:(c + 1) * 128] = (acc * inv).astype(jnp.bfloat16)

    def mlp_chunk(hn, j, acc):
        lo = j * fch
        hi = min(f, lo + fch)
        h1 = jax.lax.dot_general(hn, w1_ref[lo:hi, :], (((1,), (1,)), ((), ())),
                                 preferred_element_type=jnp.float32)
        h1 = h1 + b1_ref[:, lo:hi].astype(jnp.float32)
        e = jnp.exp(-jnp.abs(h1))
        e2 = e * e
        pos = h1 >= 0
        num = jnp.where(pos, 1.0 + 2.0 * e, e2 + 2.0 * e)
        den = num + jnp.where(pos, 2.0 * e2, 2.0)
        act = (h1 * num / den).astype(jnp.bfloat16)
        y = jnp.dot(act, w2_ref[lo:hi, :], preferred_element_type=jnp.float32)
        return acc + y

    def run(par, do_a, do_b, masked):
        wr_ref, rd_ref = bufs[par], bufs[1 - par]
        if do_a:
            if do_b:
                wr_ref[0:_HALO, d:] = rd_ref[ts:ts + _HALO, d:]
            else:
                wr_ref[0:_HALO, d:] = jnp.zeros((_HALO, 2 * d), jnp.float32)
            ln1_stage()

        def body(j, carry):
            if do_a:
                qkv_chunk(wr_ref, pl.multiple_of(j * nc, 128))
            if do_b:
                attn_block(rd_ref, pl.multiple_of(j * rb, rb), masked)
            return carry

        jax.lax.fori_loop(0, nj, body, 0)
        if do_b:
            x = xp_ref[...].astype(jnp.float32)
            h = x + jnp.dot(a_ref[...], wo_ref[...], preferred_element_type=jnp.float32)
            hn = _layernorm(h).astype(jnp.bfloat16)
            acc = h
            for j in range(nf):
                acc = mlp_chunk(hn, j, acc)
            o_ref[...] = acc.astype(o_ref.dtype)

    @pl.when(i == 0)
    def _():
        permute_weights()
        run(0, True, False, False)

    @pl.when(i == 1)
    def _():
        run(1, True, True, True)

    for par in range(2):
        @pl.when((i > 1) & (i < nt) & (i % 2 == par))
        def _():
            run(par, True, True, False)

    @pl.when(i == nt)
    def _():
        run(nt % 2, False, True, False)


@jax.jit
def pallas_sequential_preLN__sliding_local_dilated__dense_activation_mish__prompt_kernel(
    A_x: jax.Array,
    A_wqkv: jax.Array,
    A_wo: jax.Array,
    B_x: jax.Array,
    B_w1: jax.Array,
    B_b1: jax.Array,
    B_w2: jax.Array,
):
    b, s, d = A_x.shape
    f = B_w1.shape[1]
    ts = 256
    nt = s // ts
    assert b == 1 and s % ts == 0 and d == _H * _DH

    x2 = A_x.reshape(s, d)
    b1 = B_b1.reshape(1, f)

    const = lambda i: (0, 0)
    out = pl.pallas_call(
        functools.partial(_kernel, ts=ts, d=d, f=f, nt=nt),
        grid=(nt + 1,),
        in_specs=[
            pl.BlockSpec((ts, d), lambda i: (jnp.minimum(i, nt - 1), 0)),
            pl.BlockSpec((ts, d), lambda i: (jnp.maximum(i - 1, 0), 0)),
            pl.BlockSpec((d, 3 * d), const),
            pl.BlockSpec((d, d), const),
            pl.BlockSpec((f, d), const),
            pl.BlockSpec((1, f), const),
            pl.BlockSpec((f, d), const),
        ],
        out_specs=pl.BlockSpec((ts, d), lambda i: (jnp.maximum(i - 1, 0), 0)),
        out_shape=jax.ShapeDtypeStruct((s, d), A_x.dtype),
        scratch_shapes=[
            pltpu.VMEM((d, 3 * d), jnp.bfloat16),
            pltpu.VMEM((d, d), jnp.bfloat16),
            pltpu.VMEM((ts, d), jnp.bfloat16),
            pltpu.VMEM((ts + _HALO, 3 * d), jnp.float32),
            pltpu.VMEM((ts + _HALO, 3 * d), jnp.float32),
            pltpu.VMEM((ts // 4 + _HALO, 2 * d), jnp.float32),
            pltpu.VMEM((ts, d), jnp.bfloat16),
        ],
        compiler_params=pltpu.CompilerParams(
            dimension_semantics=("arbitrary",),
            vmem_limit_bytes=64 * 1024 * 1024,
        ),
    )(x2, x2, A_wqkv, A_wo, B_w1.T, b1, B_w2)
    return out.reshape(b, s, d)
```

```python
import functools

import jax
import jax.numpy as jnp
import jax.experimental.pallas as pl
import jax.experimental.pallas.tpu as pltpu

_H = 32
_DH = 16
_W = 8
_DIL = 2
_HALO = 16
_EPS = 1e-5
_NEG = -1e9


def _layernorm(x):
    m = jnp.mean(x, axis=-1, keepdims=True)
    xc = x - m
    v = jnp.mean(xc * xc, axis=-1, keepdims=True)
    return xc * jax.lax.rsqrt(v + _EPS)


def _kernel(x_ref, xp_ref, wqkv_ref, wo_in_ref, w1_ref, b1_ref, w2_ref, o_ref,
            wp_ref, wo_ref, q_ref, kv_ref, a_ref, *, ts, d, f, nt):
    i = pl.program_id(0)
    nchunk = d // 128
    rb = 32
    nrb = ts // rb
    fch = 128
    nf = -(-f // fch)

    def permute_weights():
        r = jax.lax.broadcasted_iota(jnp.int32, (d, d), 0)
        c = jax.lax.broadcasted_iota(jnp.int32, (d, d), 1)
        perm = (c == (r % _DH) * _H + r // _DH).astype(jnp.bfloat16)
        perm_t = (r == (c % _DH) * _H + c // _DH).astype(jnp.bfloat16)
        wo_ref[...] = jnp.dot(perm_t, wo_in_ref[...],
                              preferred_element_type=jnp.float32).astype(jnp.bfloat16)
        for t in range(3):
            wp_ref[:, t * d:(t + 1) * d] = jnp.dot(
                wqkv_ref[:, t * d:(t + 1) * d], perm,
                preferred_element_type=jnp.float32).astype(jnp.bfloat16)

    def qkv_stage():
        x = x_ref[...].astype(jnp.float32)
        xn = _layernorm(x).astype(jnp.bfloat16)
        qkv = jnp.dot(xn, wp_ref[...], preferred_element_type=jnp.float32)
        q_ref[...] = qkv[:, :d] * (_DH ** -0.5)
        kv_ref[_HALO:_HALO + ts, :] = qkv[:, d:]

    def attn_block(r0, masked):
        logits = []
        for w in range(_W):
            off = _HALO + r0 - w * _DIL
            acc = None
            for c in range(nchunk):
                kc = kv_ref[off:off + rb, c * 128:(c + 1) * 128]
                t = q_ref[r0:r0 + rb, c * 128:(c + 1) * 128] * kc
                acc = t if acc is None else acc + t
            acc = acc + pltpu.roll(acc, 64, 1)
            acc = acc + pltpu.roll(acc, 32, 1)
            if masked and w > 0 and r0 < w * _DIL:
                row = r0 + jax.lax.broadcasted_iota(jnp.int32, (rb, 128), 0)
                acc = jnp.where(row >= w * _DIL, acc, _NEG)
            logits.append(acc)
        m = functools.reduce(jnp.maximum, logits)
        ps = [jnp.exp(l - m) for l in logits]
        inv = 1.0 / functools.reduce(lambda a, b: a + b, ps)
        for c in range(nchunk):
            acc = None
            for w in range(_W):
                off = _HALO + r0 - w * _DIL
                vc = kv_ref[off:off + rb, d + c * 128:d + (c + 1) * 128]
                t = ps[w] * vc
                acc = t if acc is None else acc + t
            a_ref[r0:r0 + rb, c * 128:(c + 1) * 128] = (acc * inv).astype(jnp.bfloat16)

    def wo_stage():
        x = xp_ref[...].astype(jnp.float32)
        return x + jnp.dot(a_ref[...], wo_ref[...],
                           preferred_element_type=jnp.float32)

    def mlp_chunk(hn, j, acc):
        lo = j * fch
        hi = min(f, lo + fch)
        h1 = jax.lax.dot_general(hn, w1_ref[lo:hi, :], (((1,), (1,)), ((), ())),
                                 preferred_element_type=jnp.float32)
        h1 = h1 + b1_ref[:, lo:hi].astype(jnp.float32)
        e = jnp.exp(-jnp.abs(h1))
        e2 = e * e
        pos = h1 >= 0
        num = jnp.where(pos, 1.0 + 2.0 * e, e2 + 2.0 * e)
        den = num + jnp.where(pos, 2.0 * e2, 2.0)
        act = (h1 * num / den).astype(jnp.bfloat16)
        y = jnp.dot(act, w2_ref[lo:hi, :], preferred_element_type=jnp.float32)
        return acc + y

    def run(do_a, do_b, masked):
        if do_b:
            h = wo_stage()
            hn = _layernorm(h).astype(jnp.bfloat16)
        if do_a:
            qkv_stage()
        acc = h if do_b else None
        for j in range(max(nf, nrb)):
            if do_b and j < nf:
                acc = mlp_chunk(hn, j, acc)
            if do_a and j < nrb:
                attn_block(j * rb, masked)
        if do_b:
            o_ref[...] = acc.astype(o_ref.dtype)

    @pl.when(i == 0)
    def _():
        permute_weights()
        kv_ref[0:_HALO, :] = jnp.zeros((_HALO, 2 * d), jnp.float32)
        run(True, False, True)

    @pl.when((i > 0) & (i < nt))
    def _():
        kv_ref[0:_HALO, :] = kv_ref[ts:ts + _HALO, :]
        run(True, True, False)

    @pl.when(i == nt)
    def _():
        run(False, True, False)


@jax.jit
def pallas_sequential_preLN__sliding_local_dilated__dense_activation_mish__prompt_kernel(
    A_x: jax.Array,
    A_wqkv: jax.Array,
    A_wo: jax.Array,
    B_x: jax.Array,
    B_w1: jax.Array,
    B_b1: jax.Array,
    B_w2: jax.Array,
):
    b, s, d = A_x.shape
    f = B_w1.shape[1]
    ts = 512
    nt = s // ts
    assert b == 1 and s % ts == 0 and d == _H * _DH

    x2 = A_x.reshape(s, d)
    b1 = B_b1.reshape(1, f)

    const = lambda i: (0, 0)
    out = pl.pallas_call(
        functools.partial(_kernel, ts=ts, d=d, f=f, nt=nt),
        grid=(nt + 1,),
        in_specs=[
            pl.BlockSpec((ts, d), lambda i: (jnp.minimum(i, nt - 1), 0)),
            pl.BlockSpec((ts, d), lambda i: (jnp.maximum(i - 1, 0), 0)),
            pl.BlockSpec((d, 3 * d), const),
            pl.BlockSpec((d, d), const),
            pl.BlockSpec((f, d), const),
            pl.BlockSpec((1, f), const),
            pl.BlockSpec((f, d), const),
        ],
        out_specs=pl.BlockSpec((ts, d), lambda i: (jnp.maximum(i - 1, 0), 0)),
        out_shape=jax.ShapeDtypeStruct((s, d), A_x.dtype),
        scratch_shapes=[
            pltpu.VMEM((d, 3 * d), jnp.bfloat16),
            pltpu.VMEM((d, d), jnp.bfloat16),
            pltpu.VMEM((ts, d), jnp.float32),
            pltpu.VMEM((ts + _HALO, 2 * d), jnp.float32),
            pltpu.VMEM((ts, d), jnp.bfloat16),
        ],
        compiler_params=pltpu.CompilerParams(
            dimension_semantics=("arbitrary",),
            vmem_limit_bytes=64 * 1024 * 1024,
        ),
    )(x2, x2, A_wqkv, A_wo, B_w1.T, b1, B_w2)
    return out.reshape(b, s, d)
```

```python
import functools

import jax
import jax.numpy as jnp
import jax.experimental.pallas as pl
import jax.experimental.pallas.tpu as pltpu

_H = 32
_DH = 16
_W = 8
_DIL = 2
_HALO = 16
_EPS = 1e-5
_NEG = -1e9


def _layernorm(x):
    m = jnp.mean(x, axis=-1, keepdims=True)
    xc = x - m
    v = jnp.mean(xc * xc, axis=-1, keepdims=True)
    return xc * jax.lax.rsqrt(v + _EPS)


def _kernel(x_ref, xp_ref, wqkv_ref, wo_in_ref, w1_ref, b1_ref, w2_ref, o_ref,
            wp_ref, wo_ref, q_ref, kv_ref, a_ref, *, ts, d, f, nt):
    i = pl.program_id(0)
    nchunk = d // 128
    rb = 32
    nrb = ts // rb
    fch = 128
    nf = -(-f // fch)

    def permute_weights():
        r = jax.lax.broadcasted_iota(jnp.int32, (d, d), 0)
        c = jax.lax.broadcasted_iota(jnp.int32, (d, d), 1)
        perm = (c == (r % _DH) * _H + r // _DH).astype(jnp.bfloat16)
        perm_t = (r == (c % _DH) * _H + c // _DH).astype(jnp.bfloat16)
        wo_ref[...] = jnp.dot(perm_t, wo_in_ref[...],
                              preferred_element_type=jnp.float32).astype(jnp.bfloat16)
        for t in range(3):
            wp_ref[:, t * d:(t + 1) * d] = jnp.dot(
                wqkv_ref[:, t * d:(t + 1) * d], perm,
                preferred_element_type=jnp.float32).astype(jnp.bfloat16)

    def qkv_stage():
        x = x_ref[...].astype(jnp.float32)
        xn = _layernorm(x).astype(jnp.bfloat16)
        qkv = jnp.dot(xn, wp_ref[...], preferred_element_type=jnp.float32)
        q_ref[...] = qkv[:, :d] * (_DH ** -0.5)
        kv_ref[_HALO:_HALO + ts, :] = qkv[:, d:]

    def attn_block(r0, masked):
        def shifted(col, a):
            lo = _HALO + r0 - 8 - a * _DIL
            return kv_ref[lo:lo + rb + 8, col:col + 128]

        def tap(sh, w):
            s_ = sh[w % 4]
            return s_[8:8 + rb] if w < 4 else s_[0:rb]

        parts = [None] * _W
        for c in range(nchunk):
            qc = q_ref[r0:r0 + rb, c * 128:(c + 1) * 128]
            sh = [shifted(c * 128, a) for a in range(4)]
            for w in range(_W):
                t = qc * tap(sh, w)
                parts[w] = t if parts[w] is None else parts[w] + t
        logits = []
        for w in range(_W):
            acc = parts[w]
            acc = acc + pltpu.roll(acc, 64, 1)
            acc = acc + pltpu.roll(acc, 32, 1)
            if masked and w > 0 and r0 < w * _DIL:
                row = r0 + jax.lax.broadcasted_iota(jnp.int32, (rb, 128), 0)
                acc = jnp.where(row >= w * _DIL, acc, _NEG)
            logits.append(acc)
        m = functools.reduce(jnp.maximum, logits)
        ps = [jnp.exp(l - m) for l in logits]
        inv = 1.0 / functools.reduce(lambda a, b: a + b, ps)
        for c in range(nchunk):
            sh = [shifted(d + c * 128, a) for a in range(4)]
            acc = None
            for w in range(_W):
                t = ps[w] * tap(sh, w)
                acc = t if acc is None else acc + t
            a_ref[r0:r0 + rb, c * 128:(c + 1) * 128] = (acc * inv).astype(jnp.bfloat16)

    def wo_stage():
        x = xp_ref[...].astype(jnp.float32)
        return x + jnp.dot(a_ref[...], wo_ref[...],
                           preferred_element_type=jnp.float32)

    def mlp_chunk(hn, j, acc):
        lo = j * fch
        hi = min(f, lo + fch)
        h1 = jax.lax.dot_general(hn, w1_ref[lo:hi, :], (((1,), (1,)), ((), ())),
                                 preferred_element_type=jnp.float32)
        h1 = h1 + b1_ref[:, lo:hi].astype(jnp.float32)
        e = jnp.exp(-jnp.abs(h1))
        e2 = e * e
        pos = h1 >= 0
        num = jnp.where(pos, 1.0 + 2.0 * e, e2 + 2.0 * e)
        den = num + jnp.where(pos, 2.0 * e2, 2.0)
        act = (h1 * num / den).astype(jnp.bfloat16)
        y = jnp.dot(act, w2_ref[lo:hi, :], preferred_element_type=jnp.float32)
        return acc + y

    def run(do_a, do_b, masked):
        if do_b:
            h = wo_stage()
            hn = _layernorm(h).astype(jnp.bfloat16)
        if do_a:
            qkv_stage()
        acc = h if do_b else None
        for j in range(max(nf, nrb)):
            if do_b and j < nf:
                acc = mlp_chunk(hn, j, acc)
            if do_a and j < nrb:
                attn_block(j * rb, masked)
        if do_b:
            o_ref[...] = acc.astype(o_ref.dtype)

    @pl.when(i == 0)
    def _():
        permute_weights()
        kv_ref[0:_HALO, :] = jnp.zeros((_HALO, 2 * d), jnp.float32)
        run(True, False, True)

    @pl.when((i > 0) & (i < nt))
    def _():
        kv_ref[0:_HALO, :] = kv_ref[ts:ts + _HALO, :]
        run(True, True, False)

    @pl.when(i == nt)
    def _():
        run(False, True, False)


@jax.jit
def pallas_sequential_preLN__sliding_local_dilated__dense_activation_mish__prompt_kernel(
    A_x: jax.Array,
    A_wqkv: jax.Array,
    A_wo: jax.Array,
    B_x: jax.Array,
    B_w1: jax.Array,
    B_b1: jax.Array,
    B_w2: jax.Array,
):
    b, s, d = A_x.shape
    f = B_w1.shape[1]
    ts = 256
    nt = s // ts
    assert b == 1 and s % ts == 0 and d == _H * _DH

    x2 = A_x.reshape(s, d)
    b1 = B_b1.reshape(1, f)

    const = lambda i: (0, 0)
    out = pl.pallas_call(
        functools.partial(_kernel, ts=ts, d=d, f=f, nt=nt),
        grid=(nt + 1,),
        in_specs=[
            pl.BlockSpec((ts, d), lambda i: (jnp.minimum(i, nt - 1), 0)),
            pl.BlockSpec((ts, d), lambda i: (jnp.maximum(i - 1, 0), 0)),
            pl.BlockSpec((d, 3 * d), const),
            pl.BlockSpec((d, d), const),
            pl.BlockSpec((f, d), const),
            pl.BlockSpec((1, f), const),
            pl.BlockSpec((f, d), const),
        ],
        out_specs=pl.BlockSpec((ts, d), lambda i: (jnp.maximum(i - 1, 0), 0)),
        out_shape=jax.ShapeDtypeStruct((s, d), A_x.dtype),
        scratch_shapes=[
            pltpu.VMEM((d, 3 * d), jnp.bfloat16),
            pltpu.VMEM((d, d), jnp.bfloat16),
            pltpu.VMEM((ts, d), jnp.float32),
            pltpu.VMEM((ts + _HALO, 2 * d), jnp.float32),
            pltpu.VMEM((ts, d), jnp.bfloat16),
        ],
        compiler_params=pltpu.CompilerParams(
            dimension_semantics=("arbitrary",),
            vmem_limit_bytes=64 * 1024 * 1024,
        ),
    )(x2, x2, A_wqkv, A_wo, B_w1.T, b1, B_w2)
    return out.reshape(b, s, d)
```

```python
import functools

import jax
import jax.numpy as jnp
import jax.experimental.pallas as pl
import jax.experimental.pallas.tpu as pltpu

_H = 32
_DH = 16
_W = 8
_DIL = 2
_HALO = 16
_EPS = 1e-5
_NEG = -1e9


def _layernorm(x):
    m = jnp.mean(x, axis=-1, keepdims=True)
    xc = x - m
    v = jnp.mean(xc * xc, axis=-1, keepdims=True)
    return xc * jax.lax.rsqrt(v + _EPS)


def _recip(x):
    r = pl.reciprocal(x, approx=True)
    return r * (2.0 - x * r)


def _kernel(x_ref, xp_ref, wqkv_hbm, wo_in_ref, w1_hbm, b1_ref, w2_hbm, o_ref,
            wp_ref, wo_ref, q_ref, kv_ref, a_ref, w1_ref, w2_ref, wqkv_ref, sem,
            *, ts, d, f, nt):
    i = pl.program_id(0)
    nchunk = d // 128
    rb = 32
    nrb = ts // rb
    fch = 128
    nf = -(-f // fch)

    def wqkv_copy():
        return pltpu.make_async_copy(wqkv_hbm, wqkv_ref, sem.at[2])

    def permute_weights():
        r = jax.lax.broadcasted_iota(jnp.int32, (d, d), 0)
        c = jax.lax.broadcasted_iota(jnp.int32, (d, d), 1)
        perm = (c == (r % _DH) * _H + r // _DH).astype(jnp.bfloat16)
        perm_t = (r == (c % _DH) * _H + c // _DH).astype(jnp.bfloat16)
        wo_ref[...] = jnp.dot(perm_t, wo_in_ref[...],
                              preferred_element_type=jnp.float32).astype(jnp.bfloat16)
        wqkv_copy().wait()
        for t in range(3):
            wt = jnp.dot(wqkv_ref[:, t * d:(t + 1) * d], perm,
                         preferred_element_type=jnp.float32)
            if t == 0:
                wt = wt * (_DH ** -0.5)
            wp_ref[:, t * d:(t + 1) * d] = wt.astype(jnp.bfloat16)

    def qkv_stage():
        x = x_ref[...].astype(jnp.float32)
        xn = _layernorm(x).astype(jnp.bfloat16)
        qkv = jnp.dot(xn, wp_ref[...], preferred_element_type=jnp.float32)
        q_ref[...] = qkv[:, :d]
        kv_ref[_HALO:_HALO + ts, :] = qkv[:, d:]

    def attn_block(r0, masked):
        def shifted(col, a):
            win = kv_ref[r0:r0 + rb + _HALO, col:col + 128]
            return pltpu.roll(win, a * _DIL, 0) if a else win

        def tap(sh, w):
            lo = _HALO - 8 * (w // 4)
            return sh[w % 4][lo:lo + rb]

        parts = [None] * _W
        for c in range(nchunk):
            qc = q_ref[r0:r0 + rb, c * 128:(c + 1) * 128]
            sh = [shifted(c * 128, a) for a in range(4)]
            for w in range(_W):
                t = qc * tap(sh, w)
                parts[w] = t if parts[w] is None else parts[w] + t
        logits = []
        for w in range(_W):
            acc = parts[w]
            acc = acc + pltpu.roll(acc, 64, 1)
            acc = acc + pltpu.roll(acc, 32, 1)
            if masked and w > 0 and r0 < w * _DIL:
                row = r0 + jax.lax.broadcasted_iota(jnp.int32, (rb, 128), 0)
                acc = jnp.where(row >= w * _DIL, acc, _NEG)
            logits.append(acc)
        m = functools.reduce(jnp.maximum, logits)
        ps = [jnp.exp(l - m) for l in logits]
        inv = _recip(functools.reduce(lambda a, b: a + b, ps))
        for c in range(nchunk):
            sh = [shifted(d + c * 128, a) for a in range(4)]
            acc = None
            for w in range(_W):
                t = ps[w] * tap(sh, w)
                acc = t if acc is None else acc + t
            a_ref[r0:r0 + rb, c * 128:(c + 1) * 128] = (acc * inv).astype(jnp.bfloat16)

    def wo_stage():
        x = xp_ref[...].astype(jnp.float32)
        return x + jnp.dot(a_ref[...], wo_ref[...],
                           preferred_element_type=jnp.float32)

    def mlp_chunk(hn, j, acc):
        lo = j * fch
        hi = min(f, lo + fch)
        h1 = jax.lax.dot_general(hn, w1_ref[lo:hi, :], (((1,), (1,)), ((), ())),
                                 preferred_element_type=jnp.float32)
        h1 = h1 + b1_ref[lo:hi].astype(jnp.float32)[None, :]
        e = jnp.exp(jnp.minimum(h1, 30.0))
        n = e * (e + 2.0)
        act = (h1 * (n * _recip(n + 2.0))).astype(jnp.bfloat16)
        y = jnp.dot(act, w2_ref[lo:hi, :], preferred_element_type=jnp.float32)
        return acc + y

    def run(do_a, do_b, masked):
        if do_b:
            h = wo_stage()
            hn = _layernorm(h).astype(jnp.bfloat16)
        if do_a:
            qkv_stage()
        acc = h if do_b else None
        for j in range(max(nf, nrb)):
            if do_b and j < nf:
                acc = mlp_chunk(hn, j, acc)
            if do_a and j < nrb:
                attn_block(j * rb, masked)
        if do_b:
            o_ref[...] = acc.astype(o_ref.dtype)

    def mlp_weight_copies():
        return (pltpu.make_async_copy(w1_hbm, w1_ref, sem.at[0]),
                pltpu.make_async_copy(w2_hbm, w2_ref, sem.at[1]))

    @pl.when(i == 1)
    def _():
        for cp in mlp_weight_copies():
            cp.wait()

    @pl.when(i == 0)
    def _():
        wqkv_copy().start()
        for cp in mlp_weight_copies():
            cp.start()
        permute_weights()
        kv_ref[0:_HALO, :] = jnp.zeros((_HALO, 2 * d), jnp.float32)
        run(True, False, True)

    @pl.when((i > 0) & (i < nt))
    def _():
        kv_ref[0:_HALO, :] = kv_ref[ts:ts + _HALO, :]
        run(True, True, False)

    @pl.when(i == nt)
    def _():
        run(False, True, False)


@jax.jit
def pallas_sequential_preLN__sliding_local_dilated__dense_activation_mish__prompt_kernel(
    A_x: jax.Array,
    A_wqkv: jax.Array,
    A_wo: jax.Array,
    B_x: jax.Array,
    B_w1: jax.Array,
    B_b1: jax.Array,
    B_w2: jax.Array,
):
    b, s, d = A_x.shape
    f = B_w1.shape[1]
    ts = 256
    nt = s // ts
    assert b == 1 and s % ts == 0 and d == _H * _DH

    x2 = A_x.reshape(s, d)

    const = lambda i: (0, 0)
    out = pl.pallas_call(
        functools.partial(_kernel, ts=ts, d=d, f=f, nt=nt),
        grid=(nt + 1,),
        in_specs=[
            pl.BlockSpec((ts, d), lambda i: (jnp.minimum(i, nt - 1), 0)),
            pl.BlockSpec((ts, d), lambda i: (jnp.maximum(i - 1, 0), 0)),
            pl.BlockSpec(memory_space=pl.ANY),
            pl.BlockSpec((d, d), const),
            pl.BlockSpec(memory_space=pl.ANY),
            pl.BlockSpec((f,), lambda i: (0,)),
            pl.BlockSpec(memory_space=pl.ANY),
        ],
        out_specs=pl.BlockSpec((ts, d), lambda i: (jnp.maximum(i - 1, 0), 0)),
        out_shape=jax.ShapeDtypeStruct((s, d), A_x.dtype),
        scratch_shapes=[
            pltpu.VMEM((d, 3 * d), jnp.bfloat16),
            pltpu.VMEM((d, d), jnp.bfloat16),
            pltpu.VMEM((ts, d), jnp.float32),
            pltpu.VMEM((ts + _HALO, 2 * d), jnp.float32),
            pltpu.VMEM((ts, d), jnp.bfloat16),
            pltpu.VMEM((f, d), jnp.bfloat16),
            pltpu.VMEM((f, d), jnp.bfloat16),
            pltpu.VMEM((d, 3 * d), jnp.bfloat16),
            pltpu.SemaphoreType.DMA((3,)),
        ],
        compiler_params=pltpu.CompilerParams(
            dimension_semantics=("arbitrary",),
            vmem_limit_bytes=64 * 1024 * 1024,
        ),
    )(x2, x2, A_wqkv, A_wo, B_w1.T, B_b1, B_w2)
    return out.reshape(b, s, d)
```
